```python
import os as _os
_os.environ.setdefault("JAX_PLATFORMS", "cpu")
import jax
import jax.numpy as jnp

def _softmax(x, axis=-1):
    return jax.nn.softmax(x, axis=axis)
def _gelu(x):
    return jax.nn.gelu(x, approximate=True)
def _silu(x):
    return jax.nn.silu(x)
def _sigmoid(x):
    return jax.nn.sigmoid(x)
def _layernorm(x, axis=-1, eps=1e-5):
    m = jnp.mean(x, axis=axis, keepdims=True)
    v = jnp.var(x, axis=axis, keepdims=True)
    return (x - m) / jnp.sqrt(v + eps)
def _scatter_add(tgt, idx, src, axis=0):
    return tgt.at[idx].add(src)
def _segment_sum(src, seg, n):
    return jax.ops.segment_sum(src, seg, n)
class _Rng:
    def __init__(self, key):
        self._k = key
    def _next(self):
        self._k, sub = jax.random.split(self._k)
        return sub
    def normal(self, shape):
        return jax.random.normal(self._next(), shape, dtype=jnp.bfloat16)
    def randint(self, lo, hi, shape):
        return jax.random.randint(self._next(), shape, lo, hi, dtype=jnp.int32)
    def uniform(self, shape, lo=0.0, hi=1.0):
        return jax.random.uniform(self._next(), shape, jnp.bfloat16, lo, hi)
    def permutation(self, n):
        return jax.random.permutation(self._next(), n)


kernel_name = 'interleave_layers__gqa_block_cached__dense_activation_mish__decode'

def setup_inputs():
    _rng = _Rng(jax.random.key(int.from_bytes(__import__("os").urandom(4), "little")))
    _w = (lambda a: (lambda t: t.astype(jnp.bfloat16) if jnp.issubdtype(t.dtype, jnp.floating) else t)(jnp.asarray(a)))
    def _A_setup():
        B, Sq, D = 1, 1, 512
        Hq, Hkv, Sk, Dh = 32, 8, 65536, 128
        assert Hq % Hkv == 0, (Hq, Hkv)
        return {
            "x": _w((lambda *s: _rng.normal(s) * 0.05)(B, Sq, D)),
            "k_cache": _w((lambda *s: _rng.normal(s) * 1.6)(B, Hkv, Sk, Dh)),
            "v_cache": _w((lambda *s: _rng.normal(s) * 1.6)(B, Hkv, Sk, Dh)),
            "wq": _w((lambda *s: _rng.normal(s) * 1.6)(D, Hq * Dh) * (D ** -0.5)),
            "wo": _w((lambda *s: _rng.normal(s) * 1.6)(Hq * Dh, D) * ((Hq * Dh) ** -0.5)),
        }
    _A_in = _A_setup()

    def _B_setup():
        B, S, D, F = 1, 1, 512, 1792
        return {
            "x": _w((lambda *s: _rng.normal(s) * 0.05)(B, S, D)),
            "w1": _w((lambda *s: _rng.normal(s) * 0.8)(D, F) * (D ** -0.5)),
            "b1": _w((lambda *s: _rng.normal(s) * 0.8)(F)),
            "w2": _w((lambda *s: _rng.normal(s) * 0.8)(F, D) * (F ** -0.5)),
        }
    _B_in = _B_setup()

    return {
        "A_x": _A_in["x"],
        "A_k_cache": _A_in["k_cache"],
        "A_v_cache": _A_in["v_cache"],
        "A_wq": _A_in["wq"],
        "A_wo": _A_in["wo"],
        "B_x": _B_in["x"],
        "B_w1": _B_in["w1"],
        "B_b1": _B_in["b1"],
        "B_w2": _B_in["w2"],
    }

def reference(A_x, A_k_cache, A_v_cache, A_wq, A_wo, B_x, B_w1, B_b1, B_w2):
    def _A_ref(x, k_cache, v_cache, wq, wo):
        B, Sq, D = x.shape
        Hq, Dh = 32, 128
        Hkv = k_cache.shape[1]
        rep = Hq // Hkv
        q = (lambda x, *d: x.transpose(*d))((x @ wq).reshape(B, Sq, Hq, Dh), 0, 2, 1, 3)
        k = jnp.repeat(k_cache, rep, axis=1)
        v = jnp.repeat(v_cache, rep, axis=1)
        scores = jnp.einsum("bhqd,bhkd->bhqk", q, k) * (Dh ** -0.5)
        p = _softmax(scores, axis=-1)
        o = jnp.einsum("bhqk,bhkd->bhqd", p, v)
        return (lambda x, *d: x.transpose(*d))(o, 0, 2, 1, 3).reshape(B, Sq, Hq * Dh) @ wo

    def _B_ref(x, w1, b1, w2):
        h = jnp.einsum("bsd,df->bsf", x, w1) + b1
        sp = jnp.log1p(jnp.exp(-jnp.abs(h))) + jnp.where(h > 0, h, jnp.zeros_like(h))
        act = h * jnp.tanh(sp)
        return jnp.einsum("bsf,fd->bsd", act, w2)

    x = A_x
    x = x + _A_ref(_layernorm(x, axis=-1), A_k_cache, A_v_cache, A_wq, A_wo)
    x = x + _B_ref(_layernorm(x, axis=-1), B_w1, B_b1, B_w2)
    x = x + _A_ref(_layernorm(x, axis=-1), A_k_cache, A_v_cache, A_wq, A_wo)
    x = x + _B_ref(_layernorm(x, axis=-1), B_w1, B_b1, B_w2)
    return x
```

```python
import jax
import jax.numpy as jnp
from jax import lax
import jax.experimental.pallas as pl
import jax.experimental.pallas.tpu as pltpu

D_MODEL, HQ, HKV, SK, DH, FF = 512, 32, 8, 65536, 128, 1792
REP = HQ // HKV
F32, BF16 = jnp.float32, jnp.bfloat16

J = 16
NB = 14 * 128
NA = SK // J - NB
NS = HKV * J
D = 3
DK = D + 1
NWV = NS - D
NWK = NS - DK
SCALE = DH ** -0.5
_NT = (((1,), (1,)), ((), ()))
assert D * 2 * NA <= D_MODEL * HQ


def _ln(x):
    m = jnp.mean(x, axis=-1, keepdims=True)
    xc = x - m
    v = jnp.mean(xc * xc, axis=-1, keepdims=True)
    return xc / jnp.sqrt(v + 1e-5)


def _kernel(x_ref, b1_ref, k_hbm, v_hbm, wq_hbm, wo_hbm, w1_hbm, w2_hbm, out_ref,
            kres, vres, kst, vst, wq_v, wo_v, w1_v, w2_v, q_s, m_s, l_s, acc_s, y_s,
            sa, sb, sw, sq):
    def a_row(s):
        return (s // J) * SK + (s % J) * NA

    def b_row(s):
        return (s // J) * SK + J * NA + (s % J) * NB

    def ka1(s):
        return pltpu.make_async_copy(k_hbm.at[pl.ds(a_row(s), NA)], kst.at[s % DK], sa.at[0, s % D])

    def va1(s):
        return pltpu.make_async_copy(v_hbm.at[pl.ds(a_row(s), NA)], vst.at[s % D], sa.at[1, s % D])

    def kb1(s):
        return pltpu.make_async_copy(k_hbm.at[pl.ds(b_row(s), NB)], kres.at[s], sb.at[0, s % D])

    def vb1(s):
        return pltpu.make_async_copy(v_hbm.at[pl.ds(b_row(s), NB)], vres.at[s], sb.at[1, s % D])

    def reg2(s, which):
        off = (s % D) * (2 * NA) + which * NA
        if not isinstance(off, int):
            off = pl.multiple_of(off, 128)
        return wq_v.at[pl.ds(off, NA)]

    def ka2(s):
        return pltpu.make_async_copy(k_hbm.at[pl.ds(a_row(s), NA)], reg2(s, 0), sa.at[0, s % D])

    def va2(s):
        return pltpu.make_async_copy(v_hbm.at[pl.ds(a_row(s), NA)], reg2(s, 1), sa.at[1, s % D])

    def wq_cp(h):
        return pltpu.make_async_copy(wq_hbm.at[:, pl.ds(h * DH, DH)],
                                     wq_v.at[pl.ds(h * D_MODEL, D_MODEL)], sq.at[h])

    def wo_cp():
        return pltpu.make_async_copy(wo_hbm, wo_v, sw.at[0])

    def w1_cp():
        return pltpu.make_async_copy(w1_hbm, w1_v, sw.at[1])

    def w2_cp():
        return pltpu.make_async_copy(w2_hbm, w2_v, sw.at[2])

    for h in range(HQ):
        wq_cp(h).start()
    for t in range(D):
        ka1(t).start()
        kb1(t).start()
        va1(t).start()
        vb1(t).start()
    wo_cp().start()
    w1_cp().start()
    w2_cp().start()

    row_id = lax.broadcasted_iota(jnp.int32, (8, 128), 0)

    def compute_q(x, second):
        xn = _ln(x).astype(BF16)
        started = 0
        for g in range(HKV):
            qg = jnp.zeros((8, 128), F32)
            for r in range(REP):
                h = g * REP + r
                qh = jnp.dot(xn, wq_v[h * D_MODEL:(h + 1) * D_MODEL, :], preferred_element_type=F32)
                qg = jnp.where(row_id == r, qh, qg)
                if second:
                    while started < 2 * D and (started + 1) * NA <= (h + 1) * D_MODEL:
                        (ka2 if started % 2 == 0 else va2)(started // 2).start()
                        started += 1
            q_s[g] = qg.astype(BF16)
        assert started == (2 * D if second else 0)

    def init_state():
        m_s[...] = jnp.full(m_s.shape, -jnp.inf, F32)
        l_s[...] = jnp.zeros(l_s.shape, F32)
        acc_s[...] = jnp.zeros(acc_s.shape, F32)
        y_s[...] = jnp.zeros(y_s.shape, F32)

    def scores(s, ka_ref):
        g = s // J
        q = q_s[g]
        sA = lax.dot_general(q, ka_ref[...], _NT, preferred_element_type=F32) * SCALE
        sB = lax.dot_general(q, kres[s], _NT, preferred_element_type=F32) * SCALE
        return g, sA, sB

    def softmax_update(g, sA, sB):
        m = m_s[g]
        m_new = jnp.maximum(m, jnp.maximum(jnp.max(sA, axis=1, keepdims=True),
                                           jnp.max(sB, axis=1, keepdims=True)))
        alpha = jnp.exp(m - m_new)
        pA = jnp.exp(sA - m_new)
        pB = jnp.exp(sB - m_new)
        l_s[g] = (alpha * l_s[g] + jnp.sum(pA, axis=1, keepdims=True)
                  + jnp.sum(pB, axis=1, keepdims=True))
        m_s[g] = m_new
        return alpha * acc_s[g], pA.astype(BF16), pB.astype(BF16)

    def pv(p, v):
        return jnp.dot(p, v, preferred_element_type=F32)

    def head_out(g):
        og = acc_s[g] / l_s[g]
        blk = jnp.concatenate([jnp.where(row_id == r, og, 0.0).astype(BF16) for r in range(REP)],
                              axis=1)
        off = g * (REP * DH)
        if not isinstance(off, int):
            off = pl.multiple_of(off, REP * DH)
        return jnp.dot(blk, wo_v[pl.ds(off, REP * DH), :], preferred_element_type=F32)

    def epilogue(x):
        y = y_s[...] + head_out(HKV - 1)
        x1 = x + jnp.sum(y, axis=0, keepdims=True)
        h = (jnp.dot(_ln(x1).astype(BF16), w1_v[...], preferred_element_type=F32)
             + b1_ref[...].astype(F32).reshape(1, FF))
        sp = jnp.log1p(jnp.exp(-jnp.abs(h))) + jnp.maximum(h, 0.0)
        act = h * jnp.tanh(sp)
        return x1 + jnp.dot(act.astype(BF16), w2_v[...], preferred_element_type=F32)

    x0 = jnp.broadcast_to(x_ref[...].astype(F32), (8, D_MODEL))
    init_state()
    for h in range(HQ):
        wq_cp(h).wait()
    compute_q(x0, False)

    def p1(s, carry):
        ka1(s).wait()
        kb1(s).wait()
        g, sA, sB = scores(s, kst.at[s % DK])

        @pl.when(s + D < NS)
        def _():
            ka1(s + D).start()
            kb1(s + D).start()

        acc, pA, pB = softmax_update(g, sA, sB)
        va1(s).wait()
        acc = acc + pv(pA, vst[s % D])
        vb1(s).wait()
        acc_s[g] = acc + pv(pB, vres[s])

        @pl.when(s + D < NS)
        def _():
            va1(s + D).start()
            vb1(s + D).start()

        @pl.when(jnp.logical_and(s % J == J - 1, s < NS - 1))
        def _():
            @pl.when(s == J - 1)
            def _():
                wo_cp().wait()
            y_s[...] += head_out(s // J)
        return carry

    lax.fori_loop(0, NS, p1, 0)
    w1_cp().wait()
    w2_cp().wait()
    x2 = epilogue(x0)
    compute_q(x2, True)
    init_state()

    def p2r(u, carry):
        s = NWV + u
        g, sA, sB = scores(s, kst.at[s % DK])
        acc, pA, pB = softmax_update(g, sA, sB)
        acc_s[g] = acc + pv(pA, vst[s % D]) + pv(pB, vres[s])
        return carry

    lax.fori_loop(0, D, p2r, 0)

    def p2(w, carry):
        ka2(w).wait()
        g, sA, sB = scores(w, reg2(w, 0))

        @pl.when(w + D < NWK)
        def _():
            ka2(w + D).start()

        acc, pA, pB = softmax_update(g, sA, sB)
        acc = acc + pv(pB, vres[w])
        va2(w).wait()
        acc_s[g] = acc + pv(pA, reg2(w, 1)[...])

        @pl.when(w + D < NWV)
        def _():
            va2(w + D).start()

        @pl.when(w % J == J - 1)
        def _():
            y_s[...] += head_out(w // J)
        return carry

    lax.fori_loop(0, NWK, p2, 0)
    for w in range(NWK, NWV):
        g, sA, sB = scores(w, kst.at[w % DK])
        acc, pA, pB = softmax_update(g, sA, sB)
        acc = acc + pv(pB, vres[w])
        va2(w).wait()
        acc_s[g] = acc + pv(pA, reg2(w, 1)[...])

    x4 = epilogue(x2)
    out_ref[...] = x4[0:1, :].astype(out_ref.dtype)


@jax.jit
def pallas_interleave_layers__gqa_block_cached__dense_activation_mish__decode_kernel(
    A_x: jax.Array,
    A_k_cache: jax.Array,
    A_v_cache: jax.Array,
    A_wq: jax.Array,
    A_wo: jax.Array,
    B_x: jax.Array,
    B_w1: jax.Array,
    B_b1: jax.Array,
    B_w2: jax.Array,
):
    any_spec = pl.BlockSpec(memory_space=pl.ANY)
    vm = pl.BlockSpec(memory_space=pltpu.VMEM)
    out = pl.pallas_call(
        _kernel,
        out_shape=jax.ShapeDtypeStruct((1, D_MODEL), BF16),
        in_specs=[vm, vm] + [any_spec] * 6,
        out_specs=vm,
        scratch_shapes=[
            pltpu.VMEM((NS, NB, DH), BF16), pltpu.VMEM((NS, NB, DH), BF16),
            pltpu.VMEM((DK, NA, DH), BF16), pltpu.VMEM((D, NA, DH), BF16),
            pltpu.VMEM((D_MODEL * HQ, DH), BF16), pltpu.VMEM((HQ * DH, D_MODEL), BF16),
            pltpu.VMEM((D_MODEL, FF), BF16), pltpu.VMEM((FF, D_MODEL), BF16),
            pltpu.VMEM((HKV, 8, DH), BF16), pltpu.VMEM((HKV, 8, 1), F32),
            pltpu.VMEM((HKV, 8, 1), F32), pltpu.VMEM((HKV, 8, DH), F32),
            pltpu.VMEM((8, D_MODEL), F32),
            pltpu.SemaphoreType.DMA((2, D)), pltpu.SemaphoreType.DMA((2, D)),
            pltpu.SemaphoreType.DMA((3,)), pltpu.SemaphoreType.DMA((HQ,)),
        ],
        compiler_params=pltpu.CompilerParams(vmem_limit_bytes=128 * 1024 * 1024),
    )(A_x.reshape(1, D_MODEL), B_b1,
      A_k_cache.reshape(HKV * SK, DH), A_v_cache.reshape(HKV * SK, DH),
      A_wq, A_wo, B_w1, B_w2)
    return out.reshape(1, 1, D_MODEL)
```

```python
import jax
import jax.numpy as jnp
from jax import lax
import jax.experimental.pallas as pl
import jax.experimental.pallas.tpu as pltpu

D_MODEL, HQ, HKV, SK, DH, FF = 512, 32, 8, 65536, 128, 1792
REP = HQ // HKV
F32, BF16 = jnp.float32, jnp.bfloat16

J = 16
NB = 14 * 128
NA = SK // J - NB
NS = HKV * J
D = 3
DK = D + 1
NWV = NS - D
NWK = NS - DK
SCALE = DH ** -0.5
_NT = (((1,), (1,)), ((), ()))
assert D * 2 * NA <= D_MODEL * HQ


def _ln(x):
    m = jnp.mean(x, axis=-1, keepdims=True)
    xc = x - m
    v = jnp.mean(xc * xc, axis=-1, keepdims=True)
    return xc / jnp.sqrt(v + 1e-5)


def _kernel(x_hbm, b1_hbm, k_hbm, v_hbm, wq_hbm, wo_hbm, w1_hbm, w2_hbm, out_ref,
            kres, vres, kst, vst, wq_v, wo_v, w1_v, w2_v, q_s, m_s, l_s, acc_s, y_s,
            x_ref, b1_ref, sa, sb, sw, sq):
    def a_row(s):
        return (s // J) * SK + (s % J) * NA

    def b_row(s):
        return (s // J) * SK + J * NA + (s % J) * NB

    def ka1(s):
        return pltpu.make_async_copy(k_hbm.at[pl.ds(a_row(s), NA)], kst.at[s % DK], sa.at[0, s % D])

    def va1(s):
        return pltpu.make_async_copy(v_hbm.at[pl.ds(a_row(s), NA)], vst.at[s % D], sa.at[1, s % D])

    def kb1(s):
        return pltpu.make_async_copy(k_hbm.at[pl.ds(b_row(s), NB)], kres.at[s], sb.at[0, s % D])

    def vb1(s):
        return pltpu.make_async_copy(v_hbm.at[pl.ds(b_row(s), NB)], vres.at[s], sb.at[1, s % D])

    def reg2(s, which):
        off = (s % D) * (2 * NA) + which * NA
        if not isinstance(off, int):
            off = pl.multiple_of(off, 128)
        return wq_v.at[pl.ds(off, NA)]

    def ka2(s):
        return pltpu.make_async_copy(k_hbm.at[pl.ds(a_row(s), NA)], reg2(s, 0), sa.at[0, s % D])

    def va2(s):
        return pltpu.make_async_copy(v_hbm.at[pl.ds(a_row(s), NA)], reg2(s, 1), sa.at[1, s % D])

    def wq_cp(h):
        return pltpu.make_async_copy(wq_hbm.at[:, pl.ds(h * DH, DH)],
                                     wq_v.at[pl.ds(h * D_MODEL, D_MODEL)], sq.at[h])

    def wo_cp():
        return pltpu.make_async_copy(wo_hbm, wo_v, sw.at[0])

    def w1_cp():
        return pltpu.make_async_copy(w1_hbm, w1_v, sw.at[1])

    def w2_cp():
        return pltpu.make_async_copy(w2_hbm, w2_v, sw.at[2])

    def x_cp():
        return pltpu.make_async_copy(x_hbm, x_ref, sw.at[3])

    def b1_cp():
        return pltpu.make_async_copy(b1_hbm, b1_ref, sw.at[4])

    for h in range(HQ):
        wq_cp(h).start()
    x_cp().start()
    b1_cp().start()
    for t in range(D):
        ka1(t).start()
        kb1(t).start()
        va1(t).start()
        vb1(t).start()
    wo_cp().start()
    w1_cp().start()
    w2_cp().start()

    row_id = lax.broadcasted_iota(jnp.int32, (8, 128), 0)

    def compute_q(x, second):
        xn = _ln(x).astype(BF16)
        started = 0
        for g in range(HKV):
            qg = jnp.zeros((8, 128), F32)
            for r in range(REP):
                h = g * REP + r
                qh = jnp.dot(xn, wq_v[h * D_MODEL:(h + 1) * D_MODEL, :], preferred_element_type=F32)
                qg = jnp.where(row_id == r, qh, qg)
                if second:
                    while started < 2 * D and (started + 1) * NA <= (h + 1) * D_MODEL:
                        (ka2 if started % 2 == 0 else va2)(started // 2).start()
                        started += 1
            q_s[g] = qg.astype(BF16)
        assert started == (2 * D if second else 0)

    def init_state():
        m_s[...] = jnp.full(m_s.shape, -jnp.inf, F32)
        l_s[...] = jnp.zeros(l_s.shape, F32)
        acc_s[...] = jnp.zeros(acc_s.shape, F32)
        y_s[...] = jnp.zeros(y_s.shape, F32)

    def scores(s, ka_ref):
        g = s // J
        q = q_s[g]
        sA = lax.dot_general(q, ka_ref[...], _NT, preferred_element_type=F32) * SCALE
        sB = lax.dot_general(q, kres[s], _NT, preferred_element_type=F32) * SCALE
        return g, sA, sB

    def softmax_update(g, sA, sB):
        m = m_s[g]
        m_new = jnp.maximum(m, jnp.maximum(jnp.max(sA, axis=1, keepdims=True),
                                           jnp.max(sB, axis=1, keepdims=True)))
        alpha = jnp.exp(m - m_new)
        pA = jnp.exp(sA - m_new)
        pB = jnp.exp(sB - m_new)
        l_s[g] = (alpha * l_s[g] + jnp.sum(pA, axis=1, keepdims=True)
                  + jnp.sum(pB, axis=1, keepdims=True))
        m_s[g] = m_new
        return alpha * acc_s[g], pA.astype(BF16), pB.astype(BF16)

    def pv(p, v):
        return jnp.dot(p, v, preferred_element_type=F32)

    def head_out(g):
        og = acc_s[g] / l_s[g]
        blk = jnp.concatenate([jnp.where(row_id == r, og, 0.0).astype(BF16) for r in range(REP)],
                              axis=1)
        off = g * (REP * DH)
        if not isinstance(off, int):
            off = pl.multiple_of(off, REP * DH)
        return jnp.dot(blk, wo_v[pl.ds(off, REP * DH), :], preferred_element_type=F32)

    def epilogue(x):
        y = y_s[...] + head_out(HKV - 1)
        x1 = x + jnp.sum(y, axis=0, keepdims=True)
        h = (jnp.dot(_ln(x1).astype(BF16), w1_v[...], preferred_element_type=F32)
             + b1_ref[...].astype(F32).reshape(1, FF))
        sp = jnp.log1p(jnp.exp(-jnp.abs(h))) + jnp.maximum(h, 0.0)
        act = h * jnp.tanh(sp)
        return x1 + jnp.dot(act.astype(BF16), w2_v[...], preferred_element_type=F32)

    init_state()
    x_cp().wait()
    b1_cp().wait()
    x0 = jnp.broadcast_to(x_ref[...].astype(F32), (8, D_MODEL))
    for h in range(HQ):
        wq_cp(h).wait()
    compute_q(x0, False)

    def p1(s, carry):
        ka1(s).wait()
        kb1(s).wait()
        g, sA, sB = scores(s, kst.at[s % DK])

        @pl.when(s + D < NS)
        def _():
            ka1(s + D).start()
            kb1(s + D).start()

        acc, pA, pB = softmax_update(g, sA, sB)
        va1(s).wait()
        acc = acc + pv(pA, vst[s % D])
        vb1(s).wait()
        acc_s[g] = acc + pv(pB, vres[s])

        @pl.when(s + D < NS)
        def _():
            va1(s + D).start()
            vb1(s + D).start()

        @pl.when(jnp.logical_and(s % J == J - 1, s < NS - 1))
        def _():
            @pl.when(s == J - 1)
            def _():
                wo_cp().wait()
            y_s[...] += head_out(s // J)
        return carry

    lax.fori_loop(0, NS, p1, 0)
    w1_cp().wait()
    w2_cp().wait()
    x2 = epilogue(x0)
    compute_q(x2, True)
    init_state()

    def p2r(u, carry):
        s = NWV + u
        g, sA, sB = scores(s, kst.at[s % DK])
        acc, pA, pB = softmax_update(g, sA, sB)
        acc_s[g] = acc + pv(pA, vst[s % D]) + pv(pB, vres[s])
        return carry

    lax.fori_loop(0, D, p2r, 0)

    def p2(w, carry):
        ka2(w).wait()
        g, sA, sB = scores(w, reg2(w, 0))

        @pl.when(w + D < NWK)
        def _():
            ka2(w + D).start()

        acc, pA, pB = softmax_update(g, sA, sB)
        acc = acc + pv(pB, vres[w])
        va2(w).wait()
        acc_s[g] = acc + pv(pA, reg2(w, 1)[...])

        @pl.when(w + D < NWV)
        def _():
            va2(w + D).start()

        @pl.when(w % J == J - 1)
        def _():
            y_s[...] += head_out(w // J)
        return carry

    lax.fori_loop(0, NWK, p2, 0)
    for w in range(NWK, NWV):
        g, sA, sB = scores(w, kst.at[w % DK])
        acc, pA, pB = softmax_update(g, sA, sB)
        acc = acc + pv(pB, vres[w])
        va2(w).wait()
        acc_s[g] = acc + pv(pA, reg2(w, 1)[...])

    x4 = epilogue(x2)
    out_ref[...] = x4[0:1, :].astype(out_ref.dtype)


@jax.jit
def pallas_interleave_layers__gqa_block_cached__dense_activation_mish__decode_kernel(
    A_x: jax.Array,
    A_k_cache: jax.Array,
    A_v_cache: jax.Array,
    A_wq: jax.Array,
    A_wo: jax.Array,
    B_x: jax.Array,
    B_w1: jax.Array,
    B_b1: jax.Array,
    B_w2: jax.Array,
):
    any_spec = pl.BlockSpec(memory_space=pl.ANY)
    vm = pl.BlockSpec(memory_space=pltpu.VMEM)
    out = pl.pallas_call(
        _kernel,
        out_shape=jax.ShapeDtypeStruct((1, D_MODEL), BF16),
        in_specs=[any_spec] * 8,
        out_specs=vm,
        scratch_shapes=[
            pltpu.VMEM((NS, NB, DH), BF16), pltpu.VMEM((NS, NB, DH), BF16),
            pltpu.VMEM((DK, NA, DH), BF16), pltpu.VMEM((D, NA, DH), BF16),
            pltpu.VMEM((D_MODEL * HQ, DH), BF16), pltpu.VMEM((HQ * DH, D_MODEL), BF16),
            pltpu.VMEM((D_MODEL, FF), BF16), pltpu.VMEM((FF, D_MODEL), BF16),
            pltpu.VMEM((HKV, 8, DH), BF16), pltpu.VMEM((HKV, 8, 1), F32),
            pltpu.VMEM((HKV, 8, 1), F32), pltpu.VMEM((HKV, 8, DH), F32),
            pltpu.VMEM((8, D_MODEL), F32),
            pltpu.VMEM((1, D_MODEL), BF16), pltpu.VMEM((FF,), BF16),
            pltpu.SemaphoreType.DMA((2, D)), pltpu.SemaphoreType.DMA((2, D)),
            pltpu.SemaphoreType.DMA((5,)), pltpu.SemaphoreType.DMA((HQ,)),
        ],
        compiler_params=pltpu.CompilerParams(vmem_limit_bytes=128 * 1024 * 1024),
    )(A_x.reshape(1, D_MODEL), B_b1,
      A_k_cache.reshape(HKV * SK, DH), A_v_cache.reshape(HKV * SK, DH),
      A_wq, A_wo, B_w1, B_w2)
    return out.reshape(1, 1, D_MODEL)
```

```python
import jax
import jax.numpy as jnp
from jax import lax
import jax.experimental.pallas as pl
import jax.experimental.pallas.tpu as pltpu

D_MODEL, HQ, HKV, SK, DH, FF = 512, 32, 8, 65536, 128, 1792
REP = HQ // HKV
F32, BF16 = jnp.float32, jnp.bfloat16

J = 16
NB = 14 * 128
NA = SK // J - NB
NS = HKV * J
D = 3
DK = D + 1
NWV = NS - D
NWK = NS - DK
W2A = FF - 1024
SCALE = DH ** -0.5
_NT = (((1,), (1,)), ((), ()))
assert D * 2 * NA <= D_MODEL * HQ


def _ln(x):
    m = jnp.mean(x, axis=-1, keepdims=True)
    xc = x - m
    v = jnp.mean(xc * xc, axis=-1, keepdims=True)
    return xc / jnp.sqrt(v + 1e-5)


def _kernel(x_hbm, b1_hbm, k_hbm, v_hbm, wq_hbm, wo_hbm, w1_hbm, w2_hbm, out_ref,
            kres, vres, kst, vst, wq_v, wo_v, w1_v, w2_v, q_s, m_s, l_s, acc_s, y_s,
            x_ref, b1_ref, sa, sb, sw, sq):
    def a_row(s):
        return (s // J) * SK + (s % J) * NA

    def b_row(s):
        return (s // J) * SK + J * NA + (s % J) * NB

    def ka1(s):
        return pltpu.make_async_copy(k_hbm.at[pl.ds(a_row(s), NA)], kst.at[s % DK], sa.at[0, s % D])

    def va1(s):
        return pltpu.make_async_copy(v_hbm.at[pl.ds(a_row(s), NA)], vst.at[s % D], sa.at[1, s % D])

    def kb1(s):
        return pltpu.make_async_copy(k_hbm.at[pl.ds(b_row(s), NB)], kres.at[s], sb.at[0, s % D])

    def vb1(s):
        return pltpu.make_async_copy(v_hbm.at[pl.ds(b_row(s), NB)], vres.at[s], sb.at[1, s % D])

    def reg2(s, which):
        off = (s % D) * (2 * NA) + which * NA
        if not isinstance(off, int):
            off = pl.multiple_of(off, 128)
        return wq_v.at[pl.ds(off, NA)]

    def ka2(s):
        return pltpu.make_async_copy(k_hbm.at[pl.ds(a_row(s), NA)], reg2(s, 0), sa.at[0, s % D])

    def va2(s):
        return pltpu.make_async_copy(v_hbm.at[pl.ds(a_row(s), NA)], reg2(s, 1), sa.at[1, s % D])

    def wq_cp(h):
        return pltpu.make_async_copy(wq_hbm.at[:, pl.ds(h * DH, DH)],
                                     wq_v.at[pl.ds(h * D_MODEL, D_MODEL)], sq.at[h])

    def wo_cp():
        return pltpu.make_async_copy(wo_hbm, wo_v, sw.at[0])

    def w1_cp():
        return pltpu.make_async_copy(w1_hbm, w1_v, sw.at[1])

    def w2_cp():
        return pltpu.make_async_copy(w2_hbm.at[pl.ds(0, W2A)], w2_v.at[pl.ds(0, W2A)], sw.at[2])

    def w2b_cp():
        return pltpu.make_async_copy(w2_hbm.at[pl.ds(W2A, FF - W2A)],
                                     w2_v.at[pl.ds(W2A, FF - W2A)], sw.at[5])

    def x_cp():
        return pltpu.make_async_copy(x_hbm, x_ref, sw.at[3])

    def b1_cp():
        return pltpu.make_async_copy(b1_hbm, b1_ref, sw.at[4])

    for h in range(HQ):
        wq_cp(h).start()
    x_cp().start()
    b1_cp().start()
    for t in range(D):
        ka1(t).start()
        kb1(t).start()
        va1(t).start()
        vb1(t).start()
    wo_cp().start()
    w1_cp().start()
    w2_cp().start()

    row_id = lax.broadcasted_iota(jnp.int32, (8, 128), 0)

    def compute_q(x, second):
        xn = _ln(x).astype(BF16)
        started = 0
        for g in range(HKV):
            qg = jnp.zeros((8, 128), F32)
            for r in range(REP):
                h = g * REP + r
                qh = jnp.dot(xn, wq_v[h * D_MODEL:(h + 1) * D_MODEL, :], preferred_element_type=F32)
                qg = jnp.where(row_id == r, qh, qg)
                if second:
                    while started < 2 * D and (started + 1) * NA <= (h + 1) * D_MODEL:
                        (ka2 if started % 2 == 0 else va2)(started // 2).start()
                        started += 1
            q_s[g] = qg.astype(BF16)
        assert started == (2 * D if second else 0)

    def init_state():
        m_s[...] = jnp.full(m_s.shape, -jnp.inf, F32)
        l_s[...] = jnp.zeros(l_s.shape, F32)
        acc_s[...] = jnp.zeros(acc_s.shape, F32)
        y_s[...] = jnp.zeros(y_s.shape, F32)

    def scores(s, ka_ref):
        g = s // J
        q = q_s[g]
        sA = lax.dot_general(q, ka_ref[...], _NT, preferred_element_type=F32) * SCALE
        sB = lax.dot_general(q, kres[s], _NT, preferred_element_type=F32) * SCALE
        return g, sA, sB

    def softmax_update(g, sA, sB):
        m = m_s[g]
        m_new = jnp.maximum(m, jnp.maximum(jnp.max(sA, axis=1, keepdims=True),
                                           jnp.max(sB, axis=1, keepdims=True)))
        alpha = jnp.exp(m - m_new)
        pA = jnp.exp(sA - m_new)
        pB = jnp.exp(sB - m_new)
        l_s[g] = (alpha * l_s[g] + jnp.sum(pA, axis=1, keepdims=True)
                  + jnp.sum(pB, axis=1, keepdims=True))
        m_s[g] = m_new
        return alpha * acc_s[g], pA.astype(BF16), pB.astype(BF16)

    def pv(p, v):
        return jnp.dot(p, v, preferred_element_type=F32)

    def head_out(g):
        og = acc_s[g] / l_s[g]
        blk = jnp.concatenate([jnp.where(row_id == r, og, 0.0).astype(BF16) for r in range(REP)],
                              axis=1)
        off = g * (REP * DH)
        if not isinstance(off, int):
            off = pl.multiple_of(off, REP * DH)
        return jnp.dot(blk, wo_v[pl.ds(off, REP * DH), :], preferred_element_type=F32)

    def epilogue(x, first):
        y = y_s[...] + head_out(HKV - 1)
        x1 = x + jnp.sum(y, axis=0, keepdims=True)
        h = (jnp.dot(_ln(x1).astype(BF16), w1_v[...], preferred_element_type=F32)
             + b1_ref[...].astype(F32).reshape(1, FF))
        sp = jnp.log1p(jnp.exp(-jnp.abs(h))) + jnp.maximum(h, 0.0)
        act = (h * jnp.tanh(sp)).astype(BF16)
        if not first:
            return x1 + jnp.dot(act, w2_v[...], preferred_element_type=F32)
        z = x1 + jnp.dot(act[:, :W2A], w2_v[0:W2A, :], preferred_element_type=F32)
        w2b_cp().wait()
        return z + jnp.dot(act[:, W2A:], w2_v[W2A:FF, :], preferred_element_type=F32)

    init_state()
    x_cp().wait()
    b1_cp().wait()
    x0 = jnp.broadcast_to(x_ref[...].astype(F32), (8, D_MODEL))
    for h in range(HQ):
        wq_cp(h).wait()
    compute_q(x0, False)

    def p1(s, carry):
        ka1(s).wait()
        kb1(s).wait()
        g, sA, sB = scores(s, kst.at[s % DK])

        @pl.when(s + D < NS)
        def _():
            ka1(s + D).start()
            kb1(s + D).start()

        acc, pA, pB = softmax_update(g, sA, sB)
        va1(s).wait()
        acc = acc + pv(pA, vst[s % D])
        vb1(s).wait()
        acc_s[g] = acc + pv(pB, vres[s])

        @pl.when(s + D < NS)
        def _():
            va1(s + D).start()
            vb1(s + D).start()

        @pl.when(s == NS - D - 1)
        def _():
            w2b_cp().start()

        @pl.when(jnp.logical_and(s % J == J - 1, s < NS - 1))
        def _():
            @pl.when(s == J - 1)
            def _():
                wo_cp().wait()
            y_s[...] += head_out(s // J)
        return carry

    lax.fori_loop(0, NS, p1, 0)
    w1_cp().wait()
    w2_cp().wait()
    x2 = epilogue(x0, True)
    compute_q(x2, True)
    init_state()

    def p2r(u, carry):
        s = NWV + u
        g, sA, sB = scores(s, kst.at[s % DK])
        acc, pA, pB = softmax_update(g, sA, sB)
        acc_s[g] = acc + pv(pA, vst[s % D]) + pv(pB, vres[s])
        return carry

    lax.fori_loop(0, D, p2r, 0)

    def p2(w, carry):
        ka2(w).wait()
        g, sA, sB = scores(w, reg2(w, 0))

        @pl.when(w + D < NWK)
        def _():
            ka2(w + D).start()

        acc, pA, pB = softmax_update(g, sA, sB)
        acc = acc + pv(pB, vres[w])
        va2(w).wait()
        acc_s[g] = acc + pv(pA, reg2(w, 1)[...])

        @pl.when(w + D < NWV)
        def _():
            va2(w + D).start()

        @pl.when(w % J == J - 1)
        def _():
            y_s[...] += head_out(w // J)
        return carry

    lax.fori_loop(0, NWK, p2, 0)
    for w in range(NWK, NWV):
        g, sA, sB = scores(w, kst.at[w % DK])
        acc, pA, pB = softmax_update(g, sA, sB)
        acc = acc + pv(pB, vres[w])
        va2(w).wait()
        acc_s[g] = acc + pv(pA, reg2(w, 1)[...])

    x4 = epilogue(x2, False)
    out_ref[...] = x4[0:1, :].astype(out_ref.dtype)


@jax.jit
def pallas_interleave_layers__gqa_block_cached__dense_activation_mish__decode_kernel(
    A_x: jax.Array,
    A_k_cache: jax.Array,
    A_v_cache: jax.Array,
    A_wq: jax.Array,
    A_wo: jax.Array,
    B_x: jax.Array,
    B_w1: jax.Array,
    B_b1: jax.Array,
    B_w2: jax.Array,
):
    any_spec = pl.BlockSpec(memory_space=pl.ANY)
    vm = pl.BlockSpec(memory_space=pltpu.VMEM)
    out = pl.pallas_call(
        _kernel,
        out_shape=jax.ShapeDtypeStruct((1, D_MODEL), BF16),
        in_specs=[any_spec] * 8,
        out_specs=vm,
        scratch_shapes=[
            pltpu.VMEM((NS, NB, DH), BF16), pltpu.VMEM((NS, NB, DH), BF16),
            pltpu.VMEM((DK, NA, DH), BF16), pltpu.VMEM((D, NA, DH), BF16),
            pltpu.VMEM((D_MODEL * HQ, DH), BF16), pltpu.VMEM((HQ * DH, D_MODEL), BF16),
            pltpu.VMEM((D_MODEL, FF), BF16), pltpu.VMEM((FF, D_MODEL), BF16),
            pltpu.VMEM((HKV, 8, DH), BF16), pltpu.VMEM((HKV, 8, 1), F32),
            pltpu.VMEM((HKV, 8, 1), F32), pltpu.VMEM((HKV, 8, DH), F32),
            pltpu.VMEM((8, D_MODEL), F32),
            pltpu.VMEM((1, D_MODEL), BF16), pltpu.VMEM((FF,), BF16),
            pltpu.SemaphoreType.DMA((2, D)), pltpu.SemaphoreType.DMA((2, D)),
            pltpu.SemaphoreType.DMA((6,)), pltpu.SemaphoreType.DMA((HQ,)),
        ],
        compiler_params=pltpu.CompilerParams(vmem_limit_bytes=128 * 1024 * 1024),
    )(A_x.reshape(1, D_MODEL), B_b1,
      A_k_cache.reshape(HKV * SK, DH), A_v_cache.reshape(HKV * SK, DH),
      A_wq, A_wo, B_w1, B_w2)
    return out.reshape(1, 1, D_MODEL)
```

```python
import jax
import jax.numpy as jnp
from jax import lax
import jax.experimental.pallas as pl
import jax.experimental.pallas.tpu as pltpu

D_MODEL, HQ, HKV, SK, DH, FF = 512, 32, 8, 65536, 128, 1792
REP = HQ // HKV
F32, BF16 = jnp.float32, jnp.bfloat16

J = 16
NB = 14 * 128
NA = SK // J - NB
NS = HKV * J
D = 3
DK = D + 1
NWV = NS - D
NWK = NS - DK
SUBA = 128
SUBB = 112
W2A = FF - 1024
SCALE = DH ** -0.5
_NT = (((1,), (1,)), ((), ()))
assert D * 2 * NA <= D_MODEL * HQ and NA % SUBA == 0 and NB % SUBB == 0


def _ln(x):
    m = jnp.mean(x, axis=-1, keepdims=True)
    xc = x - m
    v = jnp.mean(xc * xc, axis=-1, keepdims=True)
    return xc / jnp.sqrt(v + 1e-5)


def _kernel(x_hbm, b1_hbm, k_hbm, v_hbm, wq_hbm, wo_hbm, w1_hbm, w2_hbm, out_ref,
            kres, vres, kst, vst, wq_v, wo_v, w1_v, w2_v, q_s, m_s, l_s, acc_s, y_s,
            x_ref, b1_ref, sa, sb, sw, sq):
    def a_row(s):
        return (s // J) * SK + (s % J) * NA

    def b_row(s):
        return (s // J) * SK + J * NA + (s % J) * NB

    def reg2(s, which):
        off = (s % D) * (2 * NA) + which * NA
        if not isinstance(off, int):
            off = pl.multiple_of(off, 128)
        return wq_v.at[pl.ds(off, NA)]

    def ka1(s):
        return k_hbm, a_row(s), NA, kst.at[s % DK], sa.at[0, s % D]

    def va1(s):
        return v_hbm, a_row(s), NA, vst.at[s % D], sa.at[1, s % D]

    def kb1(s):
        return k_hbm, b_row(s), NB, kres.at[s], sb.at[0, s % D]

    def vb1(s):
        return v_hbm, b_row(s), NB, vres.at[s], sb.at[1, s % D]

    def ka2(s):
        return k_hbm, a_row(s), NA, reg2(s, 0), sa.at[0, s % D]

    def va2(s):
        return v_hbm, a_row(s), NA, reg2(s, 1), sa.at[1, s % D]

    def wait(piece):
        dst, sem = piece[3], piece[4]
        pltpu.make_async_copy(dst, dst, sem).wait()

    def start_pair(kp, vp, sub):
        n = (kp if kp is not None else vp)[2] // sub
        for i in range(n):
            for piece, prio in ((kp, 0), (vp, 1)):
                if piece is not None:
                    src, row, _, dst, sem = piece
                    pltpu.make_async_copy(src.at[pl.ds(row + i * sub, sub)],
                                          dst.at[pl.ds(i * sub, sub)], sem).start(priority=prio)

    def wq_cp(h):
        return pltpu.make_async_copy(wq_hbm.at[:, pl.ds(h * DH, DH)],
                                     wq_v.at[pl.ds(h * D_MODEL, D_MODEL)], sq.at[h])

    def wo_cp():
        return pltpu.make_async_copy(wo_hbm, wo_v, sw.at[0])

    def w1_cp():
        return pltpu.make_async_copy(w1_hbm, w1_v, sw.at[1])

    def w2_cp():
        return pltpu.make_async_copy(w2_hbm.at[pl.ds(0, W2A)], w2_v.at[pl.ds(0, W2A)], sw.at[2])

    def w2b_cp():
        return pltpu.make_async_copy(w2_hbm.at[pl.ds(W2A, FF - W2A)],
                                     w2_v.at[pl.ds(W2A, FF - W2A)], sw.at[5])

    def x_cp():
        return pltpu.make_async_copy(x_hbm, x_ref, sw.at[3])

    def b1_cp():
        return pltpu.make_async_copy(b1_hbm, b1_ref, sw.at[4])

    for h in range(HQ):
        wq_cp(h).start(priority=h % 2)
    x_cp().start()
    b1_cp().start()
    for t in range(D - 1):
        start_pair(ka1(t), va1(t), SUBA)
        start_pair(kb1(t), vb1(t), SUBB)
    wo_cp().start()
    w1_cp().start()
    w2_cp().start()

    row_id = lax.broadcasted_iota(jnp.int32, (8, 128), 0)

    def compute_q(x, second):
        xn = _ln(x).astype(BF16)
        started = 0
        for g in range(HKV):
            qg = jnp.zeros((8, 128), F32)
            for r in range(REP):
                h = g * REP + r
                qh = jnp.dot(xn, wq_v[h * D_MODEL:(h + 1) * D_MODEL, :], preferred_element_type=F32)
                qg = jnp.where(row_id == r, qh, qg)
                if second:
                    while started < 2 * D and (started + 1) * NA <= (h + 1) * D_MODEL:
                        if started % 2 == 0:
                            start_pair(ka2(started // 2), None, SUBA)
                        else:
                            start_pair(None, va2(started // 2), SUBA)
                        started += 1
            q_s[g] = qg.astype(BF16)
        assert started == (2 * D if second else 0)

    def init_state():
        m_s[...] = jnp.full(m_s.shape, -jnp.inf, F32)
        l_s[...] = jnp.zeros(l_s.shape, F32)
        acc_s[...] = jnp.zeros(acc_s.shape, F32)
        y_s[...] = jnp.zeros(y_s.shape, F32)

    def scores(s, ka_ref):
        g = s // J
        q = q_s[g]
        sB = lax.dot_general(q, kres[s], _NT, preferred_element_type=F32) * SCALE
        sA = lax.dot_general(q, ka_ref[...], _NT, preferred_element_type=F32) * SCALE
        return g, sA, sB

    def softmax_update(g, sA, sB):
        m = m_s[g]
        m_new = jnp.maximum(m, jnp.maximum(jnp.max(sA, axis=1, keepdims=True),
                                           jnp.max(sB, axis=1, keepdims=True)))
        alpha = jnp.exp(m - m_new)
        pA = jnp.exp(sA - m_new)
        pB = jnp.exp(sB - m_new)
        l_s[g] = (alpha * l_s[g] + jnp.sum(pA, axis=1, keepdims=True)
                  + jnp.sum(pB, axis=1, keepdims=True))
        m_s[g] = m_new
        return alpha * acc_s[g], pA.astype(BF16), pB.astype(BF16)

    def pv(p, v):
        return jnp.dot(p, v, preferred_element_type=F32)

    def head_out(g):
        og = acc_s[g] / l_s[g]
        blk = jnp.concatenate([jnp.where(row_id == r, og, 0.0).astype(BF16) for r in range(REP)],
                              axis=1)
        off = g * (REP * DH)
        if not isinstance(off, int):
            off = pl.multiple_of(off, REP * DH)
        return jnp.dot(blk, wo_v[pl.ds(off, REP * DH), :], preferred_element_type=F32)

    def epilogue(x, first):
        y = y_s[...] + head_out(HKV - 1)
        x1 = x + jnp.sum(y, axis=0, keepdims=True)
        h = (jnp.dot(_ln(x1).astype(BF16), w1_v[...], preferred_element_type=F32)
             + b1_ref[...].astype(F32).reshape(1, FF))
        sp = jnp.log1p(jnp.exp(-jnp.abs(h))) + jnp.maximum(h, 0.0)
        act = (h * jnp.tanh(sp)).astype(BF16)
        if not first:
            return x1 + jnp.dot(act, w2_v[...], preferred_element_type=F32)
        z = x1 + jnp.dot(act[:, :W2A], w2_v[0:W2A, :], preferred_element_type=F32)
        w2b_cp().wait()
        return z + jnp.dot(act[:, W2A:], w2_v[W2A:FF, :], preferred_element_type=F32)

    init_state()
    x_cp().wait()
    b1_cp().wait()
    x0 = jnp.broadcast_to(x_ref[...].astype(F32), (8, D_MODEL))
    for h in range(HQ):
        wq_cp(h).wait()
    compute_q(x0, False)

    def p1(s, carry):
        wait(ka1(s))
        wait(kb1(s))

        @pl.when(s + 2 < NS)
        def _():
            start_pair(ka1(s + 2), va1(s + 2), SUBA)
            start_pair(kb1(s + 2), vb1(s + 2), SUBB)

        @pl.when(s == NS - 3)
        def _():
            w2b_cp().start(priority=1)

        g, sA, sB = scores(s, kst.at[s % DK])
        acc, pA, pB = softmax_update(g, sA, sB)
        wait(va1(s))
        acc = acc + pv(pA, vst[s % D])
        wait(vb1(s))
        acc_s[g] = acc + pv(pB, vres[s])

        @pl.when(jnp.logical_and(s % J == J - 1, s < NS - 1))
        def _():
            @pl.when(s == J - 1)
            def _():
                wo_cp().wait()
            y_s[...] += head_out(s // J)
        return carry

    lax.fori_loop(0, NS, p1, 0)
    w1_cp().wait()
    w2_cp().wait()
    x2 = epilogue(x0, True)
    compute_q(x2, True)
    init_state()

    def p2r(u, carry):
        s = NWV + u
        g, sA, sB = scores(s, kst.at[s % DK])
        acc, pA, pB = softmax_update(g, sA, sB)
        acc_s[g] = acc + pv(pA, vst[s % D]) + pv(pB, vres[s])
        return carry

    lax.fori_loop(0, D, p2r, 0)

    def p2(w, carry):
        wait(ka2(w))

        @pl.when(jnp.logical_and(w >= 1, w + 2 < NWK))
        def _():
            start_pair(ka2(w + 2), va2(w + 2), SUBA)

        @pl.when(w + 2 == NWK)
        def _():
            start_pair(None, va2(w + 2), SUBA)

        g, sA, sB = scores(w, reg2(w, 0))
        acc, pA, pB = softmax_update(g, sA, sB)
        acc = acc + pv(pB, vres[w])
        wait(va2(w))
        acc_s[g] = acc + pv(pA, reg2(w, 1)[...])

        @pl.when(w % J == J - 1)
        def _():
            y_s[...] += head_out(w // J)
        return carry

    lax.fori_loop(0, NWK, p2, 0)
    for w in range(NWK, NWV):
        g, sA, sB = scores(w, kst.at[w % DK])
        acc, pA, pB = softmax_update(g, sA, sB)
        acc = acc + pv(pB, vres[w])
        wait(va2(w))
        acc_s[g] = acc + pv(pA, reg2(w, 1)[...])

    x4 = epilogue(x2, False)
    out_ref[...] = x4[0:1, :].astype(out_ref.dtype)


@jax.jit
def pallas_interleave_layers__gqa_block_cached__dense_activation_mish__decode_kernel(
    A_x: jax.Array,
    A_k_cache: jax.Array,
    A_v_cache: jax.Array,
    A_wq: jax.Array,
    A_wo: jax.Array,
    B_x: jax.Array,
    B_w1: jax.Array,
    B_b1: jax.Array,
    B_w2: jax.Array,
):
    any_spec = pl.BlockSpec(memory_space=pl.ANY)
    vm = pl.BlockSpec(memory_space=pltpu.VMEM)
    out = pl.pallas_call(
        _kernel,
        out_shape=jax.ShapeDtypeStruct((1, D_MODEL), BF16),
        in_specs=[any_spec] * 8,
        out_specs=vm,
        scratch_shapes=[
            pltpu.VMEM((NS, NB, DH), BF16), pltpu.VMEM((NS, NB, DH), BF16),
            pltpu.VMEM((DK, NA, DH), BF16), pltpu.VMEM((D, NA, DH), BF16),
            pltpu.VMEM((D_MODEL * HQ, DH), BF16), pltpu.VMEM((HQ * DH, D_MODEL), BF16),
            pltpu.VMEM((D_MODEL, FF), BF16), pltpu.VMEM((FF, D_MODEL), BF16),
            pltpu.VMEM((HKV, 8, DH), BF16), pltpu.VMEM((HKV, 8, 1), F32),
            pltpu.VMEM((HKV, 8, 1), F32), pltpu.VMEM((HKV, 8, DH), F32),
            pltpu.VMEM((8, D_MODEL), F32),
            pltpu.VMEM((1, D_MODEL), BF16), pltpu.VMEM((FF,), BF16),
            pltpu.SemaphoreType.DMA((2, D)), pltpu.SemaphoreType.DMA((2, D)),
            pltpu.SemaphoreType.DMA((6,)), pltpu.SemaphoreType.DMA((HQ,)),
        ],
        compiler_params=pltpu.CompilerParams(vmem_limit_bytes=128 * 1024 * 1024),
    )(A_x.reshape(1, D_MODEL), B_b1,
      A_k_cache.reshape(HKV * SK, DH), A_v_cache.reshape(HKV * SK, DH),
      A_wq, A_wo, B_w1, B_w2)
    return out.reshape(1, 1, D_MODEL)
```

```python
import jax
import jax.numpy as jnp
from jax import lax
import jax.experimental.pallas as pl
import jax.experimental.pallas.tpu as pltpu

D_MODEL, HQ, HKV, SK, DH, FF = 512, 32, 8, 65536, 128, 1792
REP = HQ // HKV
F32, BF16 = jnp.float32, jnp.bfloat16

J = 16
NB = 14 * 128
NA = SK // J - NB
NS = HKV * J
D = 3
DK = D + 1
NWV = NS - D
NWK = NS - DK
SUBA = 128
SUBB = 112
W2A = FF - 1024
SCALE = DH ** -0.5
_NT = (((1,), (1,)), ((), ()))
assert D * 2 * NA <= D_MODEL * HQ and NA % SUBA == 0 and NB % SUBB == 0


def _ln(x):
    m = jnp.mean(x, axis=-1, keepdims=True)
    xc = x - m
    v = jnp.mean(xc * xc, axis=-1, keepdims=True)
    return xc / jnp.sqrt(v + 1e-5)


def _kernel(x_hbm, b1_hbm, k_hbm, v_hbm, wq_hbm, wo_hbm, w1_hbm, w2_hbm, out_ref,
            kres, vres, kst, vst, wq_v, wo_v, w1_v, w2_v, q_s, m_s, l_s, acc_s, y_s,
            x_ref, b1_ref, sa, sb, sw, sq):
    def a_row(s):
        return (s // J) * SK + (s % J) * NA

    def b_row(s):
        return (s // J) * SK + J * NA + (s % J) * NB

    def reg2(s, which):
        off = (s % D) * (2 * NA) + which * NA
        if not isinstance(off, int):
            off = pl.multiple_of(off, 128)
        return wq_v.at[pl.ds(off, NA)]

    def ka1(s):
        return k_hbm, a_row(s), NA, kst.at[s % DK], sa.at[0, s % D]

    def va1(s):
        return v_hbm, a_row(s), NA, vst.at[s % D], sa.at[1, s % D]

    def kb1(s):
        return k_hbm, b_row(s), NB, kres.at[s], sb.at[0, s % D]

    def vb1(s):
        return v_hbm, b_row(s), NB, vres.at[s], sb.at[1, s % D]

    def ka2(s):
        return k_hbm, a_row(s), NA, reg2(s, 0), sa.at[0, s % D]

    def va2(s):
        return v_hbm, a_row(s), NA, reg2(s, 1), sa.at[1, s % D]

    def wait(piece):
        dst, sem = piece[3], piece[4]
        pltpu.make_async_copy(dst, dst, sem).wait()

    def start_pair(kp, vp, sub):
        n = (kp if kp is not None else vp)[2] // sub
        for i in range(n):
            for piece, prio in ((kp, 0), (vp, 1)):
                if piece is not None:
                    src, row, _, dst, sem = piece
                    pltpu.make_async_copy(src.at[pl.ds(row + i * sub, sub)],
                                          dst.at[pl.ds(i * sub, sub)], sem).start(priority=prio)

    def wq_cp(h):
        return pltpu.make_async_copy(wq_hbm.at[:, pl.ds(h * DH, DH)],
                                     wq_v.at[pl.ds(h * D_MODEL, D_MODEL)], sq.at[h])

    def wo_cp():
        return pltpu.make_async_copy(wo_hbm, wo_v, sw.at[0])

    def w1_cp():
        return pltpu.make_async_copy(w1_hbm, w1_v, sw.at[1])

    def w2_cp():
        return pltpu.make_async_copy(w2_hbm.at[pl.ds(0, W2A)], w2_v.at[pl.ds(0, W2A)], sw.at[2])

    def w2b_cp():
        return pltpu.make_async_copy(w2_hbm.at[pl.ds(W2A, FF - W2A)],
                                     w2_v.at[pl.ds(W2A, FF - W2A)], sw.at[5])

    def x_cp():
        return pltpu.make_async_copy(x_hbm, x_ref, sw.at[3])

    def b1_cp():
        return pltpu.make_async_copy(b1_hbm, b1_ref, sw.at[4])

    def split_start(src, dst, sem, rows, chunk):
        for n, r in enumerate(range(0, rows, chunk)):
            pltpu.make_async_copy(src.at[pl.ds(r, chunk)], dst.at[pl.ds(r, chunk)],
                                  sem).start(priority=n % 2)

    for h in range(HQ):
        split_start(wq_hbm.at[:, pl.ds(h * DH, DH)], wq_v.at[pl.ds(h * D_MODEL, D_MODEL)],
                    sq.at[h], D_MODEL, 128)
    x_cp().start()
    b1_cp().start()
    for t in range(D - 1):
        start_pair(ka1(t), va1(t), SUBA)
        start_pair(kb1(t), vb1(t), SUBB)
    split_start(wo_hbm, wo_v, sw.at[0], HQ * DH, 32)
    split_start(w1_hbm, w1_v, sw.at[1], D_MODEL, 16)
    split_start(w2_hbm, w2_v, sw.at[2], W2A, 32)

    row_id = lax.broadcasted_iota(jnp.int32, (8, 128), 0)

    def compute_q(x, second):
        xn = _ln(x).astype(BF16)
        started = 0
        for g in range(HKV):
            qg = jnp.zeros((8, 128), F32)
            for r in range(REP):
                h = g * REP + r
                qh = jnp.dot(xn, wq_v[h * D_MODEL:(h + 1) * D_MODEL, :], preferred_element_type=F32)
                qg = jnp.where(row_id == r, qh, qg)
                if second:
                    while started < 2 * D and (started + 1) * NA <= (h + 1) * D_MODEL:
                        if started % 2 == 0:
                            start_pair(ka2(started // 2), None, SUBA)
                        else:
                            start_pair(None, va2(started // 2), SUBA)
                        started += 1
            q_s[g] = qg.astype(BF16)
        assert started == (2 * D if second else 0)

    def init_state():
        m_s[...] = jnp.full(m_s.shape, -jnp.inf, F32)
        l_s[...] = jnp.zeros(l_s.shape, F32)
        acc_s[...] = jnp.zeros(acc_s.shape, F32)
        y_s[...] = jnp.zeros(y_s.shape, F32)

    def scores(s, ka_ref):
        g = s // J
        q = q_s[g]
        sB = lax.dot_general(q, kres[s], _NT, preferred_element_type=F32) * SCALE
        sA = lax.dot_general(q, ka_ref[...], _NT, preferred_element_type=F32) * SCALE
        return g, sA, sB

    def softmax_update(g, sA, sB):
        m = m_s[g]
        m_new = jnp.maximum(m, jnp.maximum(jnp.max(sA, axis=1, keepdims=True),
                                           jnp.max(sB, axis=1, keepdims=True)))
        alpha = jnp.exp(m - m_new)
        pA = jnp.exp(sA - m_new)
        pB = jnp.exp(sB - m_new)
        l_s[g] = (alpha * l_s[g] + jnp.sum(pA, axis=1, keepdims=True)
                  + jnp.sum(pB, axis=1, keepdims=True))
        m_s[g] = m_new
        return alpha * acc_s[g], pA.astype(BF16), pB.astype(BF16)

    def pv(p, v):
        return jnp.dot(p, v, preferred_element_type=F32)

    def head_out(g):
        og = acc_s[g] / l_s[g]
        blk = jnp.concatenate([jnp.where(row_id == r, og, 0.0).astype(BF16) for r in range(REP)],
                              axis=1)
        off = g * (REP * DH)
        if not isinstance(off, int):
            off = pl.multiple_of(off, REP * DH)
        return jnp.dot(blk, wo_v[pl.ds(off, REP * DH), :], preferred_element_type=F32)

    def epilogue(x, first):
        y = y_s[...] + head_out(HKV - 1)
        x1 = x + jnp.sum(y, axis=0, keepdims=True)
        h = (jnp.dot(_ln(x1).astype(BF16), w1_v[...], preferred_element_type=F32)
             + b1_ref[...].astype(F32).reshape(1, FF))
        sp = jnp.log1p(jnp.exp(-jnp.abs(h))) + jnp.maximum(h, 0.0)
        act = (h * jnp.tanh(sp)).astype(BF16)
        if not first:
            return x1 + jnp.dot(act, w2_v[...], preferred_element_type=F32)
        z = x1 + jnp.dot(act[:, :W2A], w2_v[0:W2A, :], preferred_element_type=F32)
        w2b_cp().wait()
        return z + jnp.dot(act[:, W2A:], w2_v[W2A:FF, :], preferred_element_type=F32)

    init_state()
    x_cp().wait()
    b1_cp().wait()
    x0 = jnp.broadcast_to(x_ref[...].astype(F32), (8, D_MODEL))
    for h in range(HQ):
        wq_cp(h).wait()
    compute_q(x0, False)

    def p1(s, carry):
        wait(ka1(s))
        wait(kb1(s))

        @pl.when(s + 2 < NS)
        def _():
            start_pair(ka1(s + 2), va1(s + 2), SUBA)
            start_pair(kb1(s + 2), vb1(s + 2), SUBB)

        @pl.when(s == NS - 3)
        def _():
            w2b_cp().start(priority=1)

        g, sA, sB = scores(s, kst.at[s % DK])
        acc, pA, pB = softmax_update(g, sA, sB)
        wait(va1(s))
        acc = acc + pv(pA, vst[s % D])
        wait(vb1(s))
        acc_s[g] = acc + pv(pB, vres[s])

        @pl.when(jnp.logical_and(s % J == J - 1, s < NS - 1))
        def _():
            @pl.when(s == J - 1)
            def _():
                wo_cp().wait()
            y_s[...] += head_out(s // J)
        return carry

    lax.fori_loop(0, NS, p1, 0)
    w1_cp().wait()
    w2_cp().wait()
    x2 = epilogue(x0, True)
    compute_q(x2, True)
    init_state()

    def p2r(u, carry):
        s = NWV + u
        g, sA, sB = scores(s, kst.at[s % DK])
        acc, pA, pB = softmax_update(g, sA, sB)
        acc_s[g] = acc + pv(pA, vst[s % D]) + pv(pB, vres[s])
        return carry

    lax.fori_loop(0, D, p2r, 0)

    def p2(w, carry):
        wait(ka2(w))

        @pl.when(jnp.logical_and(w >= 1, w + 2 < NWK))
        def _():
            start_pair(ka2(w + 2), va2(w + 2), SUBA)

        @pl.when(w + 2 == NWK)
        def _():
            start_pair(None, va2(w + 2), SUBA)

        g, sA, sB = scores(w, reg2(w, 0))
        acc, pA, pB = softmax_update(g, sA, sB)
        acc = acc + pv(pB, vres[w])
        wait(va2(w))
        acc_s[g] = acc + pv(pA, reg2(w, 1)[...])

        @pl.when(w % J == J - 1)
        def _():
            y_s[...] += head_out(w // J)
        return carry

    lax.fori_loop(0, NWK, p2, 0)
    for w in range(NWK, NWV):
        g, sA, sB = scores(w, kst.at[w % DK])
        acc, pA, pB = softmax_update(g, sA, sB)
        acc = acc + pv(pB, vres[w])
        wait(va2(w))
        acc_s[g] = acc + pv(pA, reg2(w, 1)[...])

    x4 = epilogue(x2, False)
    out_ref[...] = x4[0:1, :].astype(out_ref.dtype)


@jax.jit
def pallas_interleave_layers__gqa_block_cached__dense_activation_mish__decode_kernel(
    A_x: jax.Array,
    A_k_cache: jax.Array,
    A_v_cache: jax.Array,
    A_wq: jax.Array,
    A_wo: jax.Array,
    B_x: jax.Array,
    B_w1: jax.Array,
    B_b1: jax.Array,
    B_w2: jax.Array,
):
    any_spec = pl.BlockSpec(memory_space=pl.ANY)
    vm = pl.BlockSpec(memory_space=pltpu.VMEM)
    out = pl.pallas_call(
        _kernel,
        out_shape=jax.ShapeDtypeStruct((1, D_MODEL), BF16),
        in_specs=[any_spec] * 8,
        out_specs=vm,
        scratch_shapes=[
            pltpu.VMEM((NS, NB, DH), BF16), pltpu.VMEM((NS, NB, DH), BF16),
            pltpu.VMEM((DK, NA, DH), BF16), pltpu.VMEM((D, NA, DH), BF16),
            pltpu.VMEM((D_MODEL * HQ, DH), BF16), pltpu.VMEM((HQ * DH, D_MODEL), BF16),
            pltpu.VMEM((D_MODEL, FF), BF16), pltpu.VMEM((FF, D_MODEL), BF16),
            pltpu.VMEM((HKV, 8, DH), BF16), pltpu.VMEM((HKV, 8, 1), F32),
            pltpu.VMEM((HKV, 8, 1), F32), pltpu.VMEM((HKV, 8, DH), F32),
            pltpu.VMEM((8, D_MODEL), F32),
            pltpu.VMEM((1, D_MODEL), BF16), pltpu.VMEM((FF,), BF16),
            pltpu.SemaphoreType.DMA((2, D)), pltpu.SemaphoreType.DMA((2, D)),
            pltpu.SemaphoreType.DMA((6,)), pltpu.SemaphoreType.DMA((HQ,)),
        ],
        compiler_params=pltpu.CompilerParams(vmem_limit_bytes=128 * 1024 * 1024),
    )(A_x.reshape(1, D_MODEL), B_b1,
      A_k_cache.reshape(HKV * SK, DH), A_v_cache.reshape(HKV * SK, DH),
      A_wq, A_wo, B_w1, B_w2)
    return out.reshape(1, 1, D_MODEL)
```
